```python
import os as _os
_os.environ.setdefault("JAX_PLATFORMS", "cpu")
import jax
import jax.numpy as jnp

def _softmax(x, axis=-1):
    return jax.nn.softmax(x, axis=axis)
def _gelu(x):
    return jax.nn.gelu(x, approximate=True)
def _silu(x):
    return jax.nn.silu(x)
def _sigmoid(x):
    return jax.nn.sigmoid(x)
def _layernorm(x, axis=-1, eps=1e-5):
    m = jnp.mean(x, axis=axis, keepdims=True)
    v = jnp.var(x, axis=axis, keepdims=True)
    return (x - m) / jnp.sqrt(v + eps)
def _scatter_add(tgt, idx, src, axis=0):
    return tgt.at[idx].add(src)
def _segment_sum(src, seg, n):
    return jax.ops.segment_sum(src, seg, n)
class _Rng:
    def __init__(self, key):
        self._k = key
    def _next(self):
        self._k, sub = jax.random.split(self._k)
        return sub
    def normal(self, shape):
        return jax.random.normal(self._next(), shape, dtype=jnp.bfloat16)
    def randint(self, lo, hi, shape):
        return jax.random.randint(self._next(), shape, lo, hi, dtype=jnp.int32)
    def uniform(self, shape, lo=0.0, hi=1.0):
        return jax.random.uniform(self._next(), shape, jnp.bfloat16, lo, hi)
    def permutation(self, n):
        return jax.random.permutation(self._next(), n)


kernel_name = 'parallel_sum__linear_kernel_hedgehog__dense_activation_gelu__prompt'

def setup_inputs():
    _rng = _Rng(jax.random.key(int.from_bytes(__import__("os").urandom(4), "little")))
    _w = (lambda a: (lambda t: t.astype(jnp.bfloat16) if jnp.issubdtype(t.dtype, jnp.floating) else t)(jnp.asarray(a)))
    def _A_setup():
        B, S, D, H = 1, 2048, 448, 16
        Dh = D // H
        return {
            "x": _w((lambda *s: _rng.normal(s) * 0.05)(B, S, D)),
            "wqkv": _w((lambda *s: _rng.normal(s) * 0.2)(D, 3 * D)),
            "w_phi": _w((lambda *s: _rng.normal(s) * 0.2)(H, Dh, Dh) * (Dh ** -0.5)),
            "wo": _w((lambda *s: _rng.normal(s) * 0.05)(D, D)),
        }
    _A_in = _A_setup()

    def _B_setup():
        B, S, D, F = 1, 2048, 448, 1792
        return {
            "x": _w((lambda *s: _rng.normal(s) * 0.05)(B, S, D)),
            "w1": _w((lambda *s: _rng.normal(s) * 0.2)(D, F) * (D ** -0.5)),
            "b1": _w((lambda *s: _rng.normal(s) * 0.2)(F) * 0.01),
            "w2": _w((lambda *s: _rng.normal(s) * 0.2)(F, D) * (F ** -0.5)),
            "b2": _w((lambda *s: _rng.normal(s) * 0.05)(D) * 0.01),
        }
    _B_in = _B_setup()

    return {
        "A_x": _A_in["x"],
        "A_wqkv": _A_in["wqkv"],
        "A_w_phi": _A_in["w_phi"],
        "A_wo": _A_in["wo"],
        "B_x": _B_in["x"],
        "B_w1": _B_in["w1"],
        "B_b1": _B_in["b1"],
        "B_w2": _B_in["w2"],
        "B_b2": _B_in["b2"],
    }

def reference(A_x, A_wqkv, A_w_phi, A_wo, B_x, B_w1, B_b1, B_w2, B_b2):
    def _A_ref(x, wqkv, w_phi, wo):
        B, S, D = x.shape
        H = 16; Dh = D // H
        qkv = (lambda x, *d: x.transpose(*d))((x @ wqkv).reshape(B, S, 3, H, Dh), 2, 0, 3, 1, 4)
        q, k, v = qkv[0], qkv[1], qkv[2]
        pq = jnp.einsum("bhsd,hdf->bhsf", q, w_phi)
        pk = jnp.einsum("bhsd,hdf->bhsf", k, w_phi)
        phi_q = jnp.concatenate([_softmax(pq, axis=-1), _softmax(-pq, axis=-1)], axis=-1)
        phi_k = jnp.concatenate([_softmax(pk, axis=-1), _softmax(-pk, axis=-1)], axis=-1)
        kv = jnp.einsum("bhsf,bhsd->bhfd", phi_k, v)
        z  = jnp.einsum("bhsf->bhf", phi_k)
        num = jnp.einsum("bhqf,bhfd->bhqd", phi_q, kv)
        den = jnp.einsum("bhqf,bhf->bhq", phi_q, z)[..., None] + 1e-6
        o = num / den
        return (lambda x, *d: x.transpose(*d))(o, 0, 2, 1, 3).reshape(B, S, D) @ wo

    def _B_ref(x, w1, b1, w2, b2):
        h = jnp.einsum("bsd,df->bsf", x, w1) + b1
        h = _gelu(h)
        return jnp.einsum("bsf,fd->bsd", h, w2) + b2

    x = A_x
    xn = _layernorm(x, axis=-1)
    return x + _A_ref(xn, A_wqkv, A_w_phi, A_wo) + _B_ref(xn, B_w1, B_b1, B_w2, B_b2)
```

```python
import jax
import jax.numpy as jnp
from jax import lax
import jax.experimental.pallas as pl
import jax.experimental.pallas.tpu as pltpu

S, D, H, DH, F = 2048, 448, 16, 28, 1792
DE = 512
G = 112
BF = jnp.bfloat16
F32 = jnp.float32
NT = (((1,), (1,)), ((), ()))
NN = (((1,), (0,)), ((), ()))


def _dot(a, b, dims=NN):
    return lax.dot_general(a, b, dims, preferred_element_type=F32)


def _seg(a, b_lo, b_hi, c, op):
    def r(u, w):
        t = op(op(u[:, 0:8], u[:, 8:16]), op(u[:, 16:24], w))
        red = {jnp.maximum: jnp.max, jnp.minimum: jnp.min, jnp.add: jnp.sum}[op]
        return red(t, axis=1, keepdims=True)
    return r(a, b_lo), r(c, b_hi)


def _phi(p, T):
    p = p.reshape(8, 56, T)
    a, b, c = p[:, 0:24], p[:, 24:32], p[:, 32:56]
    lo = lax.broadcasted_iota(jnp.int32, (8, 8, T), 1) < 4
    outs = []
    for sgn in (1, -1):
        if sgn == 1:
            mA, mB = _seg(a, jnp.where(lo, b, -jnp.inf), jnp.where(lo, -jnp.inf, b), c, jnp.maximum)
            ea, eb, ec = jnp.exp(a - mA), jnp.exp(b - jnp.where(lo, mA, mB)), jnp.exp(c - mB)
        else:
            mA, mB = _seg(a, jnp.where(lo, b, jnp.inf), jnp.where(lo, jnp.inf, b), c, jnp.minimum)
            ea, eb, ec = jnp.exp(mA - a), jnp.exp(jnp.where(lo, mA, mB) - b), jnp.exp(mB - c)
        sA, sB = _seg(ea, jnp.where(lo, eb, 0.0), jnp.where(lo, 0.0, eb), ec, jnp.add)
        rA, rB = 1.0 / sA, 1.0 / sB
        ph = jnp.concatenate([ea * rA, eb * jnp.where(lo, rA, rB), ec * rB], axis=1)
        outs.append(ph.reshape(D, T).astype(BF))
    return outs


def make(T=512):
    NC = S // T

    def body(x_hbm, wqkv_hbm, wphi_ref, wo_hbm, w1_hbm, b1_ref, w2T_hbm, b2_ref, o_hbm,
             x_v, wqkv_v, wo_v, w1_v, w2T, wT, woT, w1T, xn_v, kv_v, kvb_v, b2c, o_v, sems, osem):
        cp_wqkv = pltpu.make_async_copy(wqkv_hbm, wqkv_v, sems.at[0])
        cp_x = pltpu.make_async_copy(x_hbm, x_v, sems.at[1])
        cp_wo = pltpu.make_async_copy(wo_hbm, wo_v, sems.at[2])
        cp_w1 = pltpu.make_async_copy(w1_hbm, w1_v.at[0:D], sems.at[3])
        cp_w2 = pltpu.make_async_copy(w2T_hbm, w2T, sems.at[4])
        cp_wqkv.start(); cp_x.start(); cp_w1.start(); cp_w2.start(); cp_wo.start()

        ri = lax.broadcasted_iota(jnp.int32, (32, 128), 0)
        ci = lax.broadcasted_iota(jnp.int32, (32, 128), 1)
        bds = []
        for g in range(4):
            rows = []
            for a in range(4):
                wp = wphi_ref[:, 4 * g + a, :]
                sel = (ci == ri + a * DH).astype(BF)[:DH]
                rows.append(lax.dot_general(wp, sel, (((0,), (0,)), ((), ())), preferred_element_type=F32))
            bds.append(jnp.concatenate(rows, axis=0)[:, :G].astype(BF))
        w1_v[D:DE, :] = jnp.zeros((DE - D, F), BF)
        w1_v[D:D + 16, :] = jnp.where(lax.broadcasted_iota(jnp.int32, (16, F), 0) == 0,
                                      jnp.broadcast_to(b1_ref[...].reshape(1, F), (16, F)), 0).astype(BF)
        b2c[...] = jnp.broadcast_to(b2_ref[...].reshape(1, D).astype(F32), (128, D)).T
        xn_v[D:DE, :] = (lax.broadcasted_iota(jnp.int32, (DE - D, S), 0) == 0).astype(BF)
        wT[:, D:DE] = jnp.zeros((3 * D, DE - D), BF)
        cp_wqkv.wait()
        wqT = wqkv_v[...].T
        for s in range(2):
            for g in range(4):
                r0 = s * D + g * G
                wT[r0:r0 + G, 0:D] = _dot(bds[g], wqT[r0:r0 + G]).astype(BF)
        wT[2 * D:3 * D, 0:D] = wqT[2 * D:3 * D]
        kv_v[...] = jnp.zeros_like(kv_v)
        cp_x.wait()
        ones16 = jnp.ones((16, T), BF)

        def p1(c, carry):
            c0 = pl.multiple_of(c * T, T)
            x = x_v[:, pl.ds(c0, T)].astype(F32)
            m = jnp.mean(x, axis=0, keepdims=True)
            xc = x - m
            v = jnp.mean(xc * xc, axis=0, keepdims=True)
            xn_v[0:D, pl.ds(c0, T)] = (xc * lax.rsqrt(v + 1e-5)).astype(BF)
            kvT = _dot(wT[D:3 * D, :], xn_v[:, pl.ds(c0, T)])
            pp, pm = _phi(kvT[:D], T)
            vT = kvT[D:].astype(BF)
            for g in range(4):
                l = jnp.concatenate([vT[g * G:(g + 1) * G], ones16], axis=0)
                r = jnp.concatenate([pp[g * G:(g + 1) * G], pm[g * G:(g + 1) * G]], axis=0)
                kv_v[g] += _dot(l, r, NT)
            return carry
        lax.fori_loop(0, NC, p1, 0)

        rg = lax.broadcasted_iota(jnp.int32, (128, 2 * G), 0)
        rh = jnp.where(rg < G, rg // DH, rg - G)
        ch = (lax.broadcasted_iota(jnp.int32, (128, 2 * G), 1) % G) // DH
        for g in range(4):
            kvb_v[g] = jnp.where(rh == ch, kv_v[g], 0.0).astype(BF)
        cp_w1.wait()
        w1T[...] = w1_v[...].T
        cp_wo.wait()
        woT[...] = wo_v[...].T
        cp_w2.wait()

        def p2(c, carry):
            c0 = pl.multiple_of(c * T, T)
            xn = xn_v[:, pl.ds(c0, T)]
            pp, pm = _phi(_dot(wT[0:D, :], xn), T)
            os_ = []
            lo = lax.broadcasted_iota(jnp.int32, (8, T), 0) < 4
            for g in range(4):
                r = jnp.concatenate([pp[g * G:(g + 1) * G], pm[g * G:(g + 1) * G]], axis=0)
                o = _dot(kvb_v[g], r)
                rd = 1.0 / (o[G:G + 8] + 1e-6)
                d = [rd[a:a + 1] for a in range(4)]
                os_ += [o[0:24] * d[0], o[24:32] * jnp.where(lo, d[0], d[1]), o[32:56] * d[1],
                        o[56:80] * d[2], o[80:88] * jnp.where(lo, d[2], d[3]), o[88:112] * d[3]]
            oT = jnp.concatenate(os_, axis=0).astype(BF)
            hh = jax.nn.gelu(_dot(w1T[...], xn), approximate=True).astype(BF)
            yT = _dot(woT[...], oT) + _dot(w2T[...], hh)
            res = x_v[:, pl.ds(c0, T)].astype(F32) + jnp.concatenate([b2c[...]] * (T // 128), axis=1)
            o_v[:, pl.ds(c0, T)] = (yT + res).astype(BF)
            pltpu.make_async_copy(o_v.at[:, pl.ds(c0, T)], o_hbm.at[:, pl.ds(c0, T)], osem.at[c]).start()
            return carry
        lax.fori_loop(0, NC, p2, 0)
        for c in range(NC):
            pltpu.make_async_copy(o_v.at[:, pl.ds(c * T, T)], o_hbm.at[:, pl.ds(c * T, T)], osem.at[c]).wait()

    @jax.jit
    def fn(A_x, A_wqkv, A_w_phi, A_wo, B_x, B_w1, B_b1, B_w2, B_b2):
        hbm = pl.BlockSpec(memory_space=pltpu.HBM)
        vm = pl.BlockSpec(memory_space=pltpu.VMEM)
        out = pl.pallas_call(
            body,
            out_shape=jax.ShapeDtypeStruct((D, S), BF),
            in_specs=[hbm, hbm, vm, hbm, hbm, vm, hbm, vm],
            out_specs=hbm,
            scratch_shapes=[
                pltpu.VMEM((D, S), BF), pltpu.VMEM((D, 3 * D), BF), pltpu.VMEM((D, D), BF),
                pltpu.VMEM((DE, F), BF), pltpu.VMEM((D, F), BF),
                pltpu.VMEM((3 * D, DE), BF), pltpu.VMEM((D, D), BF), pltpu.VMEM((F, DE), BF),
                pltpu.VMEM((DE, S), BF), pltpu.VMEM((4, 128, 2 * G), F32), pltpu.VMEM((4, 128, 2 * G), BF),
                pltpu.VMEM((D, 128), F32), pltpu.VMEM((D, S), BF),
                pltpu.SemaphoreType.DMA((5,)), pltpu.SemaphoreType.DMA((NC,)),
            ],
            compiler_params=pltpu.CompilerParams(vmem_limit_bytes=64 * 1024 * 1024),
        )(A_x[0].T, A_wqkv, A_w_phi.transpose(1, 0, 2), A_wo, B_w1, B_b1, B_w2.T, B_b2)
        return out.T[None]
    return fn


pallas_parallel_sum__linear_kernel_hedgehog__dense_activation_gelu__prompt_kernel = make(T=512)
```

```python
import jax
import jax.numpy as jnp
from jax import lax
import jax.experimental.pallas as pl
import jax.experimental.pallas.tpu as pltpu

S, D, H, DH, F = 2048, 448, 16, 28, 1792
DE = 512
G = 112
BF = jnp.bfloat16
F32 = jnp.float32
NT = (((1,), (1,)), ((), ()))
NN = (((1,), (0,)), ((), ()))


def _dot(a, b, dims=NN):
    return lax.dot_general(a, b, dims, preferred_element_type=F32)


def _seg(a, b_lo, b_hi, c, op):
    def r(u, w):
        t = op(op(u[:, 0:8], u[:, 8:16]), op(u[:, 16:24], w))
        red = {jnp.maximum: jnp.max, jnp.minimum: jnp.min, jnp.add: jnp.sum}[op]
        return red(t, axis=1, keepdims=True)
    return r(a, b_lo), r(c, b_hi)


def _phi(p, T):
    p = p.reshape(8, 56, T)
    a, b, c = p[:, 0:24], p[:, 24:32], p[:, 32:56]
    lo = lax.broadcasted_iota(jnp.int32, (8, 8, T), 1) < 4
    outs = []
    for sgn in (1, -1):
        if sgn == 1:
            mA, mB = _seg(a, jnp.where(lo, b, -jnp.inf), jnp.where(lo, -jnp.inf, b), c, jnp.maximum)
            ea, eb, ec = jnp.exp(a - mA), jnp.exp(b - jnp.where(lo, mA, mB)), jnp.exp(c - mB)
        else:
            mA, mB = _seg(a, jnp.where(lo, b, jnp.inf), jnp.where(lo, jnp.inf, b), c, jnp.minimum)
            ea, eb, ec = jnp.exp(mA - a), jnp.exp(jnp.where(lo, mA, mB) - b), jnp.exp(mB - c)
        sA, sB = _seg(ea, jnp.where(lo, eb, 0.0), jnp.where(lo, 0.0, eb), ec, jnp.add)
        rA, rB = 1.0 / sA, 1.0 / sB
        ph = jnp.concatenate([ea * rA, eb * jnp.where(lo, rA, rB), ec * rB], axis=1)
        outs.append(ph.reshape(D, T).astype(BF))
    return outs


def make(T2=1024, P2U=False, OSUB=256, CH=(1024, 1024)):
    NC2 = S // T2; NO = S // OSUB
    NC = len(CH); CO = [sum(CH[:i]) for i in range(NC)]

    def body(x_hbm, wqkv_hbm, wphi_ref, wo_hbm, w1_hbm, b1_ref, w2T_hbm, b2_ref, o_hbm,
             x_v, wqkv_v, wo_v, w1_v, w2T, wT, woT, w1T, xn_v, kv_v, kvb_v, b2c, o_v, sems, osem, xsem):
        cp_wqkv = pltpu.make_async_copy(wqkv_hbm, wqkv_v, sems.at[0])
        cp_xs = [pltpu.make_async_copy(x_hbm.at[:, CO[c]:CO[c] + CH[c]], x_v.at[:, CO[c]:CO[c] + CH[c]], xsem.at[c]) for c in range(NC)]
        cp_wo = pltpu.make_async_copy(wo_hbm, wo_v, sems.at[2])
        cp_w1 = pltpu.make_async_copy(w1_hbm, w1_v.at[0:D], sems.at[3])
        cp_w2 = pltpu.make_async_copy(w2T_hbm, w2T, sems.at[4])
        cp_wqkv.start(); cp_xs[0].start()

        ri = lax.broadcasted_iota(jnp.int32, (32, 128), 0)
        ci = lax.broadcasted_iota(jnp.int32, (32, 128), 1)
        bds = []
        for g in range(4):
            rows = []
            for a in range(4):
                wp = wphi_ref[:, 4 * g + a, :]
                sel = (ci == ri + a * DH).astype(BF)[:DH]
                rows.append(lax.dot_general(wp, sel, (((0,), (0,)), ((), ())), preferred_element_type=F32))
            bds.append(jnp.concatenate(rows, axis=0)[:, :G].astype(BF))
        w1_v[D:DE, :] = jnp.zeros((DE - D, F), BF)
        w1_v[D:D + 16, :] = jnp.where(lax.broadcasted_iota(jnp.int32, (16, F), 0) == 0,
                                      jnp.broadcast_to(b1_ref[...].reshape(1, F), (16, F)), 0).astype(BF)
        b2c[...] = jnp.broadcast_to(b2_ref[...].reshape(1, D).astype(F32), (128, D)).T
        xn_v[D:DE, :] = (lax.broadcasted_iota(jnp.int32, (DE - D, S), 0) == 0).astype(BF)
        wT[:, D:DE] = jnp.zeros((3 * D, DE - D), BF)
        cp_wqkv.wait()
        for c in range(1, NC):
            cp_xs[c].start()
        cp_w1.start(); cp_w2.start(); cp_wo.start()
        wqT = wqkv_v[...].T
        for g in range(4):
            r0 = D + g * G
            wT[r0:r0 + G, 0:D] = _dot(bds[g], wqT[r0:r0 + G]).astype(BF)
        wT[2 * D:3 * D, 0:D] = wqT[2 * D:3 * D]
        for g in range(4):
            wT[g * G:(g + 1) * G, 0:D] = _dot(bds[g], wqT[g * G:(g + 1) * G]).astype(BF)
        kv_v[...] = jnp.zeros_like(kv_v)
        cp_xs[0].wait()

        def p1(c, carry):
            c0 = CO[c]; T = CH[c]; ones16 = jnp.ones((16, T), BF)
            if c > 0:
                cp_xs[c].wait()
            if c == NC - 1:
                cp_w1.wait()
                w1T[...] = w1_v[...].T
            x = x_v[:, pl.ds(c0, T)].astype(F32)
            m = jnp.mean(x, axis=0, keepdims=True)
            xc = x - m
            v = jnp.mean(xc * xc, axis=0, keepdims=True)
            xn_v[0:D, pl.ds(c0, T)] = (xc * lax.rsqrt(v + 1e-5)).astype(BF)
            kvT = _dot(wT[D:3 * D, :], xn_v[:, pl.ds(c0, T)])
            pp, pm = _phi(kvT[:D], T)
            vT = kvT[D:].astype(BF)
            for g in range(4):
                l = jnp.concatenate([vT[g * G:(g + 1) * G], ones16], axis=0)
                r = jnp.concatenate([pp[g * G:(g + 1) * G], pm[g * G:(g + 1) * G]], axis=0)
                kv_v[g] += _dot(r, l, NT)
            return carry
        for c in range(NC):
                p1(c, 0)

        rg = lax.broadcasted_iota(jnp.int32, (128, 2 * G), 0)
        rh = jnp.where(rg < G, rg // DH, rg - G)
        ch = (lax.broadcasted_iota(jnp.int32, (128, 2 * G), 1) % G) // DH
        for g in range(4):
            kvb_v[g] = jnp.where(rh == ch, kv_v[g].T, 0.0).astype(BF)
        cp_wo.wait()
        woT[...] = wo_v[...].T
        cp_w2.wait()

        def p2(c, carry):
            c0 = pl.multiple_of(c * T2, T2)
            xn = xn_v[:, pl.ds(c0, T2)]
            pp, pm = _phi(_dot(wT[0:D, :], xn), T2)
            os_ = []
            lo = lax.broadcasted_iota(jnp.int32, (8, T2), 0) < 4
            for g in range(4):
                r = jnp.concatenate([pp[g * G:(g + 1) * G], pm[g * G:(g + 1) * G]], axis=0)
                o = _dot(kvb_v[g], r)
                rd = 1.0 / (o[G:G + 8] + 1e-6)
                d = [rd[a:a + 1] for a in range(4)]
                os_ += [o[0:24] * d[0], o[24:32] * jnp.where(lo, d[0], d[1]), o[32:56] * d[1],
                        o[56:80] * d[2], o[80:88] * jnp.where(lo, d[2], d[3]), o[88:112] * d[3]]
            oT = jnp.concatenate(os_, axis=0).astype(BF)
            hh = jax.nn.gelu(_dot(w1T[...], xn), approximate=True).astype(BF)
            for u in range(T2 // OSUB):
                sl = slice(u * OSUB, (u + 1) * OSUB)
                cs = pl.ds(pl.multiple_of(c0 + u * OSUB, OSUB), OSUB)
                yT = _dot(woT[...], oT[:, sl]) + _dot(w2T[...], hh[:, sl])
                res = x_v[:, cs].astype(F32) + jnp.concatenate([b2c[...]] * (OSUB // 128), axis=1)
                o_v[:, cs] = (yT + res).astype(BF)
                pltpu.make_async_copy(o_v.at[:, cs], o_hbm.at[:, cs], osem.at[c * (T2 // OSUB) + u]).start()
            return carry
        if P2U:
            for c in range(NC2):
                p2(c, 0)
        else:
            lax.fori_loop(0, NC2, p2, 0)
        for c in range(NO):
            pltpu.make_async_copy(o_v.at[:, pl.ds(c * OSUB, OSUB)], o_hbm.at[:, pl.ds(c * OSUB, OSUB)], osem.at[c]).wait()

    @jax.jit
    def fn(A_x, A_wqkv, A_w_phi, A_wo, B_x, B_w1, B_b1, B_w2, B_b2):
        hbm = pl.BlockSpec(memory_space=pltpu.HBM)
        vm = pl.BlockSpec(memory_space=pltpu.VMEM)
        out = pl.pallas_call(
            body,
            out_shape=jax.ShapeDtypeStruct((D, S), BF),
            in_specs=[hbm, hbm, vm, hbm, hbm, vm, hbm, vm],
            out_specs=hbm,
            scratch_shapes=[
                pltpu.VMEM((D, S), BF), pltpu.VMEM((D, 3 * D), BF), pltpu.VMEM((D, D), BF),
                pltpu.VMEM((DE, F), BF), pltpu.VMEM((D, F), BF),
                pltpu.VMEM((3 * D, DE), BF), pltpu.VMEM((D, D), BF), pltpu.VMEM((F, DE), BF),
                pltpu.VMEM((DE, S), BF), pltpu.VMEM((4, 2 * G, 128), F32), pltpu.VMEM((4, 128, 2 * G), BF),
                pltpu.VMEM((D, 128), F32), pltpu.VMEM((D, S), BF),
                pltpu.SemaphoreType.DMA((5,)), pltpu.SemaphoreType.DMA((NO,)), pltpu.SemaphoreType.DMA((NC,)),
            ],
            compiler_params=pltpu.CompilerParams(vmem_limit_bytes=64 * 1024 * 1024),
        )(A_x[0].T, A_wqkv, A_w_phi.transpose(1, 0, 2), A_wo, B_w1, B_b1, B_w2.T, B_b2)
        return out.T[None]
    return fn


pallas_parallel_sum__linear_kernel_hedgehog__dense_activation_gelu__prompt_kernel = make()
```

```python
import jax
import jax.numpy as jnp
from jax import lax
import jax.experimental.pallas as pl
import jax.experimental.pallas.tpu as pltpu

S, D, H, DH, F = 2048, 448, 16, 28, 1792
DE = 512
G = 112
BF = jnp.bfloat16
F32 = jnp.float32
NT = (((1,), (1,)), ((), ()))
NN = (((1,), (0,)), ((), ()))


def _dot(a, b, dims=NN):
    return lax.dot_general(a, b, dims, preferred_element_type=F32)


def _sA(a11, a12, a21, a22):
    return [t.astype(BF) for t in (a11 + a22, a21 + a22, a11, a22, a11 + a12, a21 - a11, a12 - a22)]


def _sB(b11, b12, b21, b22):
    return [t.astype(BF) for t in (b11 + b22, b11, b12 - b22, b21 - b11, b22, b11 + b12, b21 + b22)]


def _seg(a, b_lo, b_hi, c, op):
    def r(u, w):
        t = op(op(u[:, 0:8], u[:, 8:16]), op(u[:, 16:24], w))
        red = {jnp.maximum: jnp.max, jnp.minimum: jnp.min, jnp.add: jnp.sum}[op]
        return red(t, axis=1, keepdims=True)
    return r(a, b_lo), r(c, b_hi)


def _phi(p, T):
    p = p.reshape(8, 56, T)
    a, b, c = p[:, 0:24], p[:, 24:32], p[:, 32:56]
    lo = lax.broadcasted_iota(jnp.int32, (8, 8, T), 1) < 4
    outs = []
    for sgn in (1, -1):
        if sgn == 1:
            mA, mB = _seg(a, jnp.where(lo, b, -jnp.inf), jnp.where(lo, -jnp.inf, b), c, jnp.maximum)
            ea, eb, ec = jnp.exp(a - mA), jnp.exp(b - jnp.where(lo, mA, mB)), jnp.exp(c - mB)
        else:
            mA, mB = _seg(a, jnp.where(lo, b, jnp.inf), jnp.where(lo, jnp.inf, b), c, jnp.minimum)
            ea, eb, ec = jnp.exp(mA - a), jnp.exp(jnp.where(lo, mA, mB) - b), jnp.exp(mB - c)
        sA, sB = _seg(ea, jnp.where(lo, eb, 0.0), jnp.where(lo, 0.0, eb), ec, jnp.add)
        rA, rB = 1.0 / sA, 1.0 / sB
        ph = jnp.concatenate([ea * rA, eb * jnp.where(lo, rA, rB), ec * rB], axis=1)
        outs.append(ph)
    return jnp.concatenate(outs, axis=1).astype(BF)


def make(T2=1024, P2U=False, OSUB=256, CH=(1024, 1024), KVS=True, S1=True, S2=True):
    NC2 = S // T2; NO = 4 * NC2
    NC = len(CH); CO = [sum(CH[:i]) for i in range(NC)]

    def body(x_hbm, wqkv_hbm, wphi_ref, wo_hbm, w1_hbm, b1_ref, w2T_hbm, b2_ref, o_hbm,
             x_v, wqkv_v, wo_v, w1_v, w2T, wT, woT, w1T, xn_v, kv_v, kvb_v, b2c, o_v, a1_v, a2_v, xb_v, sems, osem, xsem):
        cp_wqkv = pltpu.make_async_copy(wqkv_hbm, wqkv_v, sems.at[0])
        cp_xs = [pltpu.make_async_copy(x_hbm.at[:, CO[c]:CO[c] + CH[c]], x_v.at[:, CO[c]:CO[c] + CH[c]], xsem.at[c]) for c in range(NC)]
        cp_wo = pltpu.make_async_copy(wo_hbm, wo_v, sems.at[2])
        cp_w1 = pltpu.make_async_copy(w1_hbm, w1_v.at[0:D], sems.at[3])
        cp_w2 = pltpu.make_async_copy(w2T_hbm, w2T, sems.at[4])
        cp_wqkv.start(); cp_xs[0].start()

        ri = lax.broadcasted_iota(jnp.int32, (32, 128), 0)
        ci = lax.broadcasted_iota(jnp.int32, (32, 128), 1)
        bds = []
        for g in range(4):
            rows = []
            for a in range(4):
                wp = wphi_ref[:, 4 * g + a, :]
                sel = (ci == ri + a * DH).astype(BF)[:DH]
                rows.append(lax.dot_general(wp, sel, (((0,), (0,)), ((), ())), preferred_element_type=F32))
            bds.append(jnp.concatenate(rows, axis=0)[:, :G].astype(BF))
        w1_v[D:DE, :] = jnp.zeros((DE - D, F), BF)
        w1_v[D:D + 16, :] = jnp.where(lax.broadcasted_iota(jnp.int32, (16, F), 0) == 0,
                                      jnp.broadcast_to(b1_ref[...].reshape(1, F), (16, F)), 0).astype(BF)
        b2c[...] = jnp.broadcast_to(b2_ref[...].reshape(1, D).astype(F32), (128, D)).T
        xn_v[D:DE, :] = (lax.broadcasted_iota(jnp.int32, (DE - D, S), 0) == 0).astype(BF)
        wT[:, D:DE] = jnp.zeros((3 * D, DE - D), BF)
        cp_wqkv.wait()
        for c in range(1, NC):
            cp_xs[c].start()
        cp_w1.start(); cp_w2.start(); cp_wo.start()
        wqT = wqkv_v[...].T
        for g in range(4):
            r0 = D + g * G
            wT[r0:r0 + G, 0:D] = _dot(bds[g], wqT[r0:r0 + G]).astype(BF)
        wT[2 * D:3 * D, 0:D] = wqT[2 * D:3 * D]
        for g in range(4):
            wT[g * G:(g + 1) * G, 0:D] = _dot(bds[g], wqT[g * G:(g + 1) * G]).astype(BF)
        kv_v[...] = jnp.zeros_like(kv_v)
        cp_xs[0].wait()

        def p1(c, carry):
            c0 = CO[c]; T = CH[c]
            if c > 0:
                cp_xs[c].wait()
            if c == NC - 1:
                cp_w1.wait()
                if S1:
                    wt = w1_v[...].T.astype(F32)
                    for i, t in enumerate(_sA(wt[:F // 2, :DE // 2], wt[:F // 2, DE // 2:], wt[F // 2:, :DE // 2], wt[F // 2:, DE // 2:])):
                        a1_v[i] = t
                else:
                    w1T[...] = w1_v[...].T
            x = x_v[:, pl.ds(c0, T)].astype(F32)
            m = jnp.mean(x, axis=0, keepdims=True)
            xc = x - m
            v = jnp.mean(xc * xc, axis=0, keepdims=True)
            xnf = xc * lax.rsqrt(v + 1e-5)
            xn_v[0:D, pl.ds(c0, T)] = xnf.astype(BF)
            if S1:
                xe = jnp.concatenate([xnf, (lax.broadcasted_iota(jnp.int32, (DE - D, T), 0) == 0).astype(F32)], axis=0)
                hT, hK = T // 2, DE // 2
                for i, t in enumerate(_sB(xe[:hK, :hT], xe[:hK, hT:], xe[hK:, :hT], xe[hK:, hT:])):
                    xb_v[i, :, c0 // 2:c0 // 2 + hT] = t
            kvT = _dot(wT[D:3 * D, :], xn_v[:, pl.ds(c0, T)])
            ph = _phi(kvT[:D], T)
            v3 = jnp.concatenate([kvT[D:].reshape(8, 56, T), jnp.ones((8, 8, T), F32)], axis=1).astype(BF)
            for g in range(8):
                if KVS:
                    kv_v[g] += _dot(v3[g], ph[g], NT)
                else:
                    kv_v[g] += _dot(ph[g], v3[g], NT)
            return carry
        for c in range(NC):
                p1(c, 0)

        rg = lax.broadcasted_iota(jnp.int32, (64, G), 0)
        rh = jnp.where(rg < 56, rg // DH, rg - 56)
        ch = (lax.broadcasted_iota(jnp.int32, (64, G), 1) % 56) // DH
        for g in range(8):
            kvb_v[g] = jnp.where(rh == ch, kv_v[g] if KVS else kv_v[g].T, 0.0).astype(BF)
        cp_wo.wait()
        woT[...] = wo_v[...].T
        cp_w2.wait()
        if S2:
            wt = w2T[...].astype(F32)
            for i, t in enumerate(_sA(wt[:D // 2, :F // 2], wt[:D // 2, F // 2:], wt[D // 2:, :F // 2], wt[D // 2:, F // 2:])):
                a2_v[i] = t

        def p2(c, carry):
            c0 = pl.multiple_of(c * T2, T2)
            xn = xn_v[:, pl.ds(c0, T2)]
            ph = _phi(_dot(wT[0:D, :], xn), T2)
            os_ = []
            lo = lax.broadcasted_iota(jnp.int32, (8, T2), 0) < 4
            for g in range(8):
                o = _dot(kvb_v[g], ph[g])
                rd = 1.0 / (o[56:64] + 1e-6)
                d0, d1 = rd[0:1], rd[1:2]
                os_ += [o[0:24] * d0, o[24:32] * jnp.where(lo, d0, d1), o[32:56] * d1]
            oT = jnp.concatenate(os_, axis=0).astype(BF)
            hT, hF, hD = T2 // 2, F // 2, D // 2
            gelu = lambda t: jax.nn.gelu(t, approximate=True)
            if S1:
                ch_ = pl.ds(pl.multiple_of(c * hT, hT), hT)
                m = [_dot(a1_v[i], xb_v[i, :, ch_]) for i in range(7)]
                h11, h12 = gelu(m[0] + m[3] - m[4] + m[6]), gelu(m[2] + m[4])
                h21, h22 = gelu(m[1] + m[3]), gelu(m[0] - m[1] + m[2] + m[5])
            else:
                hh = gelu(_dot(w1T[...], xn))
                h11, h12, h21, h22 = hh[:hF, :hT], hh[:hF, hT:], hh[hF:, :hT], hh[hF:, hT:]

            def emit(i, j, y):
                rs = slice(i * hD, (i + 1) * hD)
                cs = pl.ds(pl.multiple_of(c0 + j * hT, hT), hT)
                y = y + _dot(woT[rs, :], oT[:, j * hT:(j + 1) * hT])
                res = x_v[rs, cs].astype(F32) + jnp.concatenate([b2c[rs, :]] * (hT // 128), axis=1)
                o_v[rs, cs] = (y + res).astype(BF)
                pltpu.make_async_copy(o_v.at[rs, cs], o_hbm.at[rs, cs], osem.at[c * 4 + i * 2 + j]).start()
            if S2:
                bb = _sB(h11, h12, h21, h22)
                mm = lambda i: _dot(a2_v[i], bb[i])
                m3, m5 = mm(2), mm(4)
                emit(0, 1, m3 + m5)
                m2, m4 = mm(1), mm(3)
                emit(1, 0, m2 + m4)
                m1 = mm(0)
                emit(0, 0, m1 + m4 - m5 + mm(6))
                emit(1, 1, m1 - m2 + m3 + mm(5))
            else:
                for j, hb in enumerate((jnp.concatenate([h11, h21], 0).astype(BF), jnp.concatenate([h12, h22], 0).astype(BF))):
                    for i in range(2):
                        emit(i, j, _dot(w2T[i * hD:(i + 1) * hD, :], hb))
            return carry
        if P2U:
            for c in range(NC2):
                p2(c, 0)
        else:
            lax.fori_loop(0, NC2, p2, 0)
        for c in range(NC2):
            for i in range(2):
                for j in range(2):
                    rs, cs = pl.ds(i * (D // 2), D // 2), pl.ds(c * T2 + j * (T2 // 2), T2 // 2)
                    pltpu.make_async_copy(o_v.at[rs, cs], o_hbm.at[rs, cs], osem.at[c * 4 + i * 2 + j]).wait()

    @jax.jit
    def fn(A_x, A_wqkv, A_w_phi, A_wo, B_x, B_w1, B_b1, B_w2, B_b2):
        hbm = pl.BlockSpec(memory_space=pltpu.HBM)
        vm = pl.BlockSpec(memory_space=pltpu.VMEM)
        out = pl.pallas_call(
            body,
            out_shape=jax.ShapeDtypeStruct((D, S), BF),
            in_specs=[hbm, hbm, vm, hbm, hbm, vm, hbm, vm],
            out_specs=hbm,
            scratch_shapes=[
                pltpu.VMEM((D, S), BF), pltpu.VMEM((D, 3 * D), BF), pltpu.VMEM((D, D), BF),
                pltpu.VMEM((DE, F), BF), pltpu.VMEM((D, F), BF),
                pltpu.VMEM((3 * D, DE), BF), pltpu.VMEM((D, D), BF), pltpu.VMEM((F, DE), BF),
                pltpu.VMEM((DE, S), BF), pltpu.VMEM((8, 64, G) if KVS else (8, G, 64), F32), pltpu.VMEM((8, 64, G), BF),
                pltpu.VMEM((D, 128), F32), pltpu.VMEM((D, S), BF),
                pltpu.VMEM((7, F // 2, DE // 2), BF), pltpu.VMEM((7, D // 2, F // 2), BF), pltpu.VMEM((7, DE // 2, S // 2), BF),
                pltpu.SemaphoreType.DMA((5,)), pltpu.SemaphoreType.DMA((NO,)), pltpu.SemaphoreType.DMA((NC,)),
            ],
            compiler_params=pltpu.CompilerParams(vmem_limit_bytes=64 * 1024 * 1024),
        )(A_x[0].T, A_wqkv, A_w_phi.transpose(1, 0, 2), A_wo, B_w1, B_b1, B_w2.T, B_b2)
        return out.T[None]
    return fn


pallas_parallel_sum__linear_kernel_hedgehog__dense_activation_gelu__prompt_kernel = make()
```
